```python
import jax
import jax.numpy as jnp

def _softmax(x, axis=-1):
    return jax.nn.softmax(x, axis=axis)
def _gelu(x):
    return jax.nn.gelu(x, approximate=True)
def _silu(x):
    return jax.nn.silu(x)
def _sigmoid(x):
    return jax.nn.sigmoid(x)
def _layernorm(x, axis=-1, eps=1e-5):
    m = jnp.mean(x, axis=axis, keepdims=True)
    v = jnp.var(x, axis=axis, keepdims=True)
    return (x - m) / jnp.sqrt(v + eps)
def _scatter_add(tgt, idx, src, axis=0):
    return tgt.at[idx].add(src)
def _segment_sum(src, seg, n):
    return jax.ops.segment_sum(src, seg, n)
class _Rng:
    def __init__(self, key):
        self._k = key
    def _next(self):
        self._k, sub = jax.random.split(self._k)
        return sub
    def normal(self, shape):
        return jax.random.normal(self._next(), shape, dtype=jnp.bfloat16)
    def randint(self, lo, hi, shape):
        return jax.random.randint(self._next(), shape, lo, hi, dtype=jnp.int32)
    def uniform(self, shape, lo=0.0, hi=1.0):
        return jax.random.uniform(self._next(), shape, jnp.bfloat16, lo, hi)
    def permutation(self, n):
        return jax.random.permutation(self._next(), n)


kernel_name = 'recurrent_scan__mha_block_cached__moe_arch_mod__decode'

def setup_inputs():
    _rng = _Rng(jax.random.key(int.from_bytes(__import__("os").urandom(4), "little")))
    _w = (lambda a: (lambda t: t.astype(jnp.bfloat16) if jnp.issubdtype(t.dtype, jnp.floating) else t)(jnp.asarray(a)))
    def _A_setup():
        B, Sq, D = 2, 1, 512
        H, Sk, Dh = 32, 16384, 128
        return {
            "x": _w((lambda *s: _rng.normal(s) * 0.05)(B, Sq, D)),
            "k_cache": _w((lambda *s: _rng.normal(s) * 0.05)(B, H, Sk, Dh)),
            "v_cache": _w((lambda *s: _rng.normal(s) * 0.05)(B, H, Sk, Dh)),
            "wq": _w((lambda *s: _rng.normal(s) * 0.05)(D, H * Dh) * (D ** -0.5)),
            "wo": _w((lambda *s: _rng.normal(s) * 0.05)(H * Dh, D) * ((H * Dh) ** -0.5)),
        }
    _A_in = _A_setup()

    def _B_setup():
        B, S, D, F, C = 2, 1, 512, 1792, 1
        return {
            "x": _w((lambda *s: _rng.normal(s) * 0.05)(B, S, D)),
            "w_r": _w((lambda *s: _rng.normal(s) * 0.05)(D)),
            "w_gate": _w((lambda *s: _rng.normal(s) * 0.05)(D, F)),
            "w_up": _w((lambda *s: _rng.normal(s) * 0.05)(D, F)),
            "w_down": _w((lambda *s: _rng.normal(s) * 0.05)(F, D)),
        }
    _B_in = _B_setup()

    return {
        "A_x": _A_in["x"],
        "A_k_cache": _A_in["k_cache"],
        "A_v_cache": _A_in["v_cache"],
        "A_wq": _A_in["wq"],
        "A_wo": _A_in["wo"],
        "B_x": _B_in["x"],
        "B_w_r": _B_in["w_r"],
        "B_w_gate": _B_in["w_gate"],
        "B_w_up": _B_in["w_up"],
        "B_w_down": _B_in["w_down"],
    }

def reference(A_x, A_k_cache, A_v_cache, A_wq, A_wo, B_x, B_w_r, B_w_gate, B_w_up, B_w_down):
    def _A_ref(x, k_cache, v_cache, wq, wo):
        B, Sq, D = x.shape
        H, Dh = 32, 128
        q = (lambda x, *d: x.transpose(*d))((x @ wq).reshape(B, Sq, H, Dh), 0, 2, 1, 3)
        scores = jnp.einsum("bhqd,bhkd->bhqk", q, k_cache) * (Dh ** -0.5)
        p = _softmax(scores, axis=-1)
        o = jnp.einsum("bhqk,bhkd->bhqd", p, v_cache)
        return (lambda x, *d: x.transpose(*d))(o, 0, 2, 1, 3).reshape(B, Sq, H * Dh) @ wo

    def _B_ref(x, w_r, w_gate, w_up, w_down):
        B, S, D = x.shape
        C = 1
        r = x @ w_r
        idx = jnp.argsort(-r, axis=-1)[:, :C]
        idx_e = jnp.repeat(idx.reshape(B, C, 1), D, axis=2)
        x_sel = jnp.take_along_axis(x, idx_e, axis=1)
        g = _silu(x_sel @ w_gate)
        u = x_sel @ w_up
        y = (g * u) @ w_down
        r_sel = _sigmoid(jnp.take_along_axis(r, idx, axis=1))
        y = y * r_sel.reshape(B, C, 1)
        b_off = (jnp.arange(B) * S).reshape(B, 1)
        flat_idx = (idx + b_off).reshape(B * C)
        zero = (x * 0.0).reshape(B * S, D)
        upd = _scatter_add(zero, flat_idx, y.reshape(B * C, D), axis=0)
        return x + upd.reshape(B, S, D)

    x = A_x
    xn = _layernorm(x, axis=-1)
    s = _A_ref(xn, A_k_cache, A_v_cache, A_wq, A_wo)
    g = _silu(_B_ref(xn, B_w_r, B_w_gate, B_w_up, B_w_down))
    return x + s * g
```

```python
import jax
import jax.numpy as jnp
from jax import lax
import jax.experimental.pallas as pl
import jax.experimental.pallas.tpu as pltpu

F32 = jnp.float32
BF16 = jnp.bfloat16

CH = 64
NR = 4
REPS = 4
NBUF = 5
PRIO = (0, 0, 1, 1)
ROWS = 8


@jax.jit
def pallas_recurrent_scan__mha_block_cached__moe_arch_mod__decode_kernel(
    A_x: jax.Array,
    A_k_cache: jax.Array,
    A_v_cache: jax.Array,
    A_wq: jax.Array,
    A_wo: jax.Array,
    B_x: jax.Array,
    B_w_r: jax.Array,
    B_w_gate: jax.Array,
    B_w_up: jax.Array,
    B_w_down: jax.Array,
):
    del B_x
    B, Sq, D = A_x.shape
    _, H, Sk, Dh = A_k_cache.shape
    F = B_w_gate.shape[1]
    assert Sq == 1 and B == 2 and Dh == 128 and D % 128 == 0

    L = REPS * CH
    RL = Sk // NR
    NC = RL // L
    T = H * NC
    CK = NR * L
    LOOK = NBUF - 1
    assert NC * CK == Sk and T >= LOOK
    scale = Dh ** -0.5
    dmas = [(j, a, b, r) for j in range(REPS) for r in range(NR)
            for b in range(B) for a in range(2)]

    def kernel(x_hbm, k_hbm, v_hbm, wq_hbm, wo_hbm, wr_hbm, wg_hbm, wu_hbm, wd_hbm,
               out_ref,
               x_vm, wr_vm, wq_vm, wo_vm, wg_vm, wu_vm, wd_vm, kvbuf, q_scr,
               wsem, sem):
        srcs = (k_hbm, v_hbm)

        def start(t, slot):
            base = (t // NC) * Sk + (t % NC) * L
            for i, (j, a, b, r) in enumerate(dmas):
                row = base + (b * H * Sk + r * RL + j * CH)
                if not isinstance(row, int):
                    row = pl.multiple_of(row, CH)
                pltpu.make_async_copy(
                    srcs[a].at[pl.ds(row, CH)],
                    kvbuf.at[slot, a, b, pl.ds(r * L + j * CH, CH)],
                    sem.at[slot],
                ).start(priority=PRIO[i % len(PRIO)])

        def wait(slot):
            pltpu.make_async_copy(kvbuf.at[slot], kvbuf.at[slot], sem.at[slot]).wait()

        cp = [pltpu.make_async_copy(s, d, wsem.at[i]) for i, (s, d) in enumerate(
            [(x_hbm, x_vm), (wq_hbm, wq_vm), (wr_hbm, wr_vm), (wg_hbm, wg_vm),
             (wu_hbm, wu_vm), (wd_hbm, wd_vm), (wo_hbm, wo_vm)])]
        cp_x, cp_wq, cp_wr, cp_wg, cp_wu, cp_wd, cp_wo = cp
        for c in cp:
            c.start()
        start(0, 0)

        cp_x.wait()
        x = x_vm[...].astype(F32)
        xc = x - jnp.mean(x, axis=-1, keepdims=True)
        var = jnp.mean(xc * xc, axis=-1, keepdims=True)
        xn = xc / jnp.sqrt(var + 1e-5)
        xn = jnp.concatenate([xn, jnp.zeros((ROWS - B, D), F32)], axis=0)
        xnb = xn.astype(BF16)

        cp_wq.wait()
        for h in range(H):
            q_scr[h] = jnp.dot(xnb, wq_vm[:, h * Dh:(h + 1) * Dh],
                               preferred_element_type=F32)

        cp_wr.wait()
        wr = wr_vm[...].astype(F32)
        racc = xn[:, 0:128] * wr[0:1, :]
        for j in range(1, D // 128):
            racc = racc + xn[:, j * 128:(j + 1) * 128] * wr[j:j + 1, :]
        r = jnp.sum(racc, axis=-1, keepdims=True)
        cp_wg.wait()
        gate = jnp.dot(xnb, wg_vm[...], preferred_element_type=F32)
        gate = gate * jax.nn.sigmoid(gate)
        cp_wu.wait()
        up = jnp.dot(xnb, wu_vm[...], preferred_element_type=F32)
        cp_wd.wait()
        y = jnp.dot((gate * up).astype(BF16), wd_vm[...], preferred_element_type=F32)
        y = y * jax.nn.sigmoid(r)
        z = xn + (xn * 0.0 + y)
        g = z * jax.nn.sigmoid(z)

        def prefetch(t, carry):
            start(t, t)
            return carry

        lax.fori_loop(1, LOOK, prefetch, 0)
        cp_wo.wait()

        nt = (((1,), (1,)), ((), ()))

        def head(h, s_acc):
            q = q_scr[h].astype(BF16)

            def step(c, carry):
                m, l, acc = carry
                t = h * NC + c
                slot = t % NBUF
                wait(slot)
                s0 = lax.dot_general(q, kvbuf[slot, 0, 0], nt, preferred_element_type=F32)
                s1 = lax.dot_general(q, kvbuf[slot, 0, 1], nt, preferred_element_type=F32)
                row = lax.broadcasted_iota(jnp.int32, (ROWS, CK), 0)
                s = jnp.where(row == 0, s0, s1) * scale
                m_new = jnp.maximum(m, jnp.max(s, axis=-1, keepdims=True))
                alpha = jnp.exp(m - m_new)
                p = jnp.exp(s - m_new)
                l = alpha * l + jnp.sum(p, axis=-1, keepdims=True)
                pb = p.astype(BF16)
                pv0 = jnp.dot(pb, kvbuf[slot, 1, 0], preferred_element_type=F32)
                pv1 = jnp.dot(pb, kvbuf[slot, 1, 1], preferred_element_type=F32)
                row = lax.broadcasted_iota(jnp.int32, (ROWS, Dh), 0)
                acc = alpha * acc + jnp.where(row == 0, pv0, pv1)

                @pl.when(t + LOOK < T)
                def _():
                    start(t + LOOK, (t + LOOK) % NBUF)

                return m_new, l, acc

            init = (jnp.full((ROWS, 1), -jnp.inf, F32), jnp.zeros((ROWS, 1), F32),
                    jnp.zeros((ROWS, Dh), F32))
            _, l, acc = lax.fori_loop(0, NC, step, init)
            wo_h = wo_vm[pl.ds(pl.multiple_of(h * Dh, Dh), Dh), :]
            return s_acc + jnp.dot((acc / l).astype(BF16), wo_h,
                                   preferred_element_type=F32)

        s_acc = lax.fori_loop(0, H, head, jnp.zeros((ROWS, D), F32))
        out_ref[...] = (x + (s_acc * g)[0:B]).astype(out_ref.dtype)

    hbm = pl.BlockSpec(memory_space=pltpu.HBM)
    out = pl.pallas_call(
        kernel,
        out_shape=jax.ShapeDtypeStruct((B * Sq, D), A_x.dtype),
        in_specs=[hbm] * 9,
        out_specs=pl.BlockSpec(memory_space=pltpu.VMEM),
        scratch_shapes=[
            pltpu.VMEM((B * Sq, D), A_x.dtype),
            pltpu.VMEM((D // 128, 128), B_w_r.dtype),
            pltpu.VMEM(A_wq.shape, A_wq.dtype),
            pltpu.VMEM(A_wo.shape, A_wo.dtype),
            pltpu.VMEM(B_w_gate.shape, B_w_gate.dtype),
            pltpu.VMEM(B_w_up.shape, B_w_up.dtype),
            pltpu.VMEM(B_w_down.shape, B_w_down.dtype),
            pltpu.VMEM((NBUF, 2, B, CK, Dh), A_k_cache.dtype),
            pltpu.VMEM((H, ROWS, Dh), F32),
            pltpu.SemaphoreType.DMA((7,)),
            pltpu.SemaphoreType.DMA((NBUF,)),
        ],
        compiler_params=pltpu.CompilerParams(vmem_limit_bytes=32 * 1024 * 1024),
        name="mha_mod_decode",
    )(
        A_x.reshape(B * Sq, D),
        A_k_cache.reshape(B * H * Sk, Dh),
        A_v_cache.reshape(B * H * Sk, Dh),
        A_wq,
        A_wo,
        B_w_r.reshape(D // 128, 128),
        B_w_gate,
        B_w_up,
        B_w_down,
    )
    return out.reshape(B, Sq, D)
```

```python
import jax
import jax.numpy as jnp
from jax import lax
import jax.experimental.pallas as pl
import jax.experimental.pallas.tpu as pltpu

F32 = jnp.float32
BF16 = jnp.bfloat16

NR = 4
PC = 32
L = 256
ROT = 1
NBUF = 9
WIT = 32
WS = 4
ROWS = 8


@jax.jit
def pallas_recurrent_scan__mha_block_cached__moe_arch_mod__decode_kernel(
    A_x: jax.Array,
    A_k_cache: jax.Array,
    A_v_cache: jax.Array,
    A_wq: jax.Array,
    A_wo: jax.Array,
    B_x: jax.Array,
    B_w_r: jax.Array,
    B_w_gate: jax.Array,
    B_w_up: jax.Array,
    B_w_down: jax.Array,
):
    del B_x
    B, Sq, D = A_x.shape
    _, H, Sk, Dh = A_k_cache.shape
    F = B_w_gate.shape[1]
    assert Sq == 1 and B <= ROWS and Dh == 128 and D % 128 == 0

    RL = Sk // NR
    NC = RL // L
    T = H * NC
    CK = NR * L
    LOOK = NBUF - 1
    NW = H // WS
    assert NC * CK == Sk and NW * WS == H and NW <= LOOK <= T
    assert D % (16 * WIT) == 0 and F % (8 * WIT) == 0 and F % 128 == 0
    scale = Dh ** -0.5

    def kernel(x_hbm, k_hbm, v_hbm, wq_hbm, wo_hbm, wr_hbm, wg_hbm, wu_hbm, wd_hbm,
               out_ref,
               x_vm, wr_vm, wq_vm, wg_vm, wu_vm, wd_vm, wo_vm, kv_vm, q_scr, o_scr,
               wsem, osem, kvsem):

        def wait_filled(buf, sem):
            pltpu.make_async_copy(buf, buf, sem).wait()

        def start_kv(t, slot):
            g0 = (t // NC) * NR
            for j in range(L // PC):
                for b in range(B):
                    row = ((t + b * ROT) % NC) * L + j * PC
                    if not isinstance(row, int):
                        row = pl.multiple_of(row, PC)
                    for a, src in enumerate((k_hbm, v_hbm)):
                        pltpu.make_async_copy(
                            src.at[b, pl.ds(g0, NR), pl.ds(row, PC)],
                            kv_vm.at[slot, a, b, :, pl.ds(j * PC, PC)],
                            kvsem.at[slot],
                        ).start(priority=a)

        def start_wo(i):
            for j in range(Dh // 8):
                row = pl.multiple_of(i * Dh + j * 8, 8)
                pltpu.make_async_copy(
                    wo_hbm.at[:, pl.ds(row, 8)],
                    wo_vm.at[i, :, pl.ds(j * 8, 8)],
                    osem.at[i],
                ).start(priority=j % 2)

        pltpu.make_async_copy(x_hbm, x_vm, wsem.at[0]).start()
        pltpu.make_async_copy(wr_hbm, wr_vm, wsem.at[1]).start(priority=1)

        def start_weights(it, carry):
            n = 0
            for src, dst, si, ns, nc in ((wq_hbm, wq_vm, 2, 2, 2), (wg_hbm, wg_vm, 3, 2, 1),
                                         (wu_hbm, wu_vm, 4, 2, 1), (wd_hbm, wd_vm, 5, 1, 2)):
                rows = src.shape[0] // (ns * WIT)
                cols = src.shape[1] // nc
                for c in range(nc):
                    for u in range(ns):
                        r0 = pl.multiple_of((u * WIT + it) * rows, 8)
                        idx = (pl.ds(r0, rows), pl.ds(c * cols, cols))
                        pltpu.make_async_copy(
                            src.at[idx], dst.at[idx], wsem.at[si]).start(priority=n % 2)
                        n += 1
            return carry

        lax.fori_loop(0, WIT, start_weights, 0)

        pending = list(range(LOOK))

        def prefetch():
            if pending:
                t = pending.pop(0)
                start_kv(t, t)

        prefetch()
        wait_filled(x_vm, wsem.at[0])
        x = x_vm[...].astype(F32)
        xc = x - jnp.mean(x, axis=-1, keepdims=True)
        var = jnp.mean(xc * xc, axis=-1, keepdims=True)
        xn = xc / jnp.sqrt(var + 1e-5)
        xn = jnp.concatenate([xn, jnp.zeros((ROWS - B, D), F32)], axis=0)
        xnb = xn.astype(BF16)
        wait_filled(wr_vm, wsem.at[1])
        wr = wr_vm[...].astype(F32)
        racc = xn[:, 0:128] * wr[0:1, :]
        for j in range(1, D // 128):
            racc = racc + xn[:, j * 128:(j + 1) * 128] * wr[j:j + 1, :]
        r = jnp.sum(racc, axis=-1, keepdims=True)
        prefetch()

        wait_filled(wq_vm, wsem.at[2])
        for h in range(H):
            q_scr[h] = jnp.dot(xnb, wq_vm[:, h * Dh:(h + 1) * Dh],
                               preferred_element_type=F32)
            if (h + 1) % (H // 2) == 0:
                prefetch()

        wait_filled(wg_vm, wsem.at[3])
        gate = jnp.dot(xnb, wg_vm[...], preferred_element_type=F32)
        gate = gate * jax.nn.sigmoid(gate)
        prefetch()
        wait_filled(wu_vm, wsem.at[4])
        up = jnp.dot(xnb, wu_vm[...], preferred_element_type=F32)
        prefetch()
        wait_filled(wd_vm, wsem.at[5])
        y = jnp.dot((gate * up).astype(BF16), wd_vm[...], preferred_element_type=F32)
        y = y * jax.nn.sigmoid(r)
        z = xn + (xn * 0.0 + y)
        g = z * jax.nn.sigmoid(z)
        while pending:
            prefetch()

        def per_batch(f):
            out = f(0)
            row = lax.broadcasted_iota(jnp.int32, out.shape, 0)
            for b in range(1, B):
                out = jnp.where(row == b, f(b), out)
            return out

        def head(h, carry):
            q = q_scr[h].astype(BF16)

            def step(c, mla):
                m, l, acc = mla
                t = h * NC + c
                slot = t % NBUF
                wait_filled(kv_vm.at[slot], kvsem.at[slot])
                s = per_batch(lambda b: lax.dot_general(
                    q, kv_vm[slot, 0, b].reshape(CK, Dh), (((1,), (1,)), ((), ())),
                    preferred_element_type=F32)) * scale
                m_new = jnp.maximum(m, jnp.max(s, axis=-1, keepdims=True))
                m_sub = jnp.where(m_new == -jnp.inf, 0.0, m_new)
                alpha = jnp.exp(m - m_sub)
                p = jnp.exp(s - m_sub)
                l = alpha * l + jnp.sum(p, axis=-1, keepdims=True)
                pb = p.astype(BF16)
                acc = alpha * acc + per_batch(lambda b: jnp.dot(
                    pb, kv_vm[slot, 1, b].reshape(CK, Dh), preferred_element_type=F32))

                nxt = t + LOOK

                @pl.when(nxt < T)
                def _():
                    start_kv(nxt, nxt % NBUF)

                @pl.when(jnp.logical_and(nxt >= T, nxt < T + NW))
                def _():
                    start_wo(nxt - T)

                return m_new, l, acc

            init = (jnp.full((ROWS, 1), -jnp.inf, F32), jnp.zeros((ROWS, 1), F32),
                    jnp.zeros((ROWS, Dh), F32))
            _, l, acc = lax.fori_loop(0, NC, step, init)
            o_scr[h] = acc / l
            return carry

        lax.fori_loop(0, H, head, 0)

        def project(i, s_acc):
            wait_filled(wo_vm.at[i], osem.at[i])
            for u in range(WS):
                s_acc = s_acc + jnp.dot(o_scr[u * NW + i].astype(BF16), wo_vm[i, u],
                                        preferred_element_type=F32)
            return s_acc

        s_acc = lax.fori_loop(0, NW, project, jnp.zeros((ROWS, D), F32))
        out_ref[...] = (x + (s_acc * g)[0:B]).astype(out_ref.dtype)

    hbm = pl.BlockSpec(memory_space=pltpu.HBM)
    out = pl.pallas_call(
        kernel,
        out_shape=jax.ShapeDtypeStruct((B * Sq, D), A_x.dtype),
        in_specs=[hbm] * 9,
        out_specs=pl.BlockSpec(memory_space=pltpu.VMEM),
        scratch_shapes=[
            pltpu.VMEM((B * Sq, D), A_x.dtype),
            pltpu.VMEM((D // 128, 128), B_w_r.dtype),
            pltpu.VMEM(A_wq.shape, A_wq.dtype),
            pltpu.VMEM(B_w_gate.shape, B_w_gate.dtype),
            pltpu.VMEM(B_w_up.shape, B_w_up.dtype),
            pltpu.VMEM(B_w_down.shape, B_w_down.dtype),
            pltpu.VMEM((NW, WS, Dh, D), A_wo.dtype),
            pltpu.VMEM((NBUF, 2, B, NR, L, Dh), A_k_cache.dtype),
            pltpu.VMEM((H, ROWS, Dh), F32),
            pltpu.VMEM((H, ROWS, Dh), F32),
            pltpu.SemaphoreType.DMA((6,)),
            pltpu.SemaphoreType.DMA((NW,)),
            pltpu.SemaphoreType.DMA((NBUF,)),
        ],
        compiler_params=pltpu.CompilerParams(vmem_limit_bytes=40 * 1024 * 1024),
        name="mha_mod_decode",
    )(
        A_x.reshape(B * Sq, D),
        A_k_cache.reshape(B, H * NR, RL, Dh),
        A_v_cache.reshape(B, H * NR, RL, Dh),
        A_wq,
        A_wo.reshape(WS, NW * Dh, D),
        B_w_r.reshape(D // 128, 128),
        B_w_gate,
        B_w_up,
        B_w_down,
    )
    return out.reshape(B, Sq, D)
```
